```python
import os as _os
_os.environ.setdefault("JAX_PLATFORMS", "cpu")
import jax
import jax.numpy as jnp

def _softmax(x, axis=-1):
    return jax.nn.softmax(x, axis=axis)
def _gelu(x):
    return jax.nn.gelu(x, approximate=True)
def _silu(x):
    return jax.nn.silu(x)
def _sigmoid(x):
    return jax.nn.sigmoid(x)
def _layernorm(x, axis=-1, eps=1e-5):
    m = jnp.mean(x, axis=axis, keepdims=True)
    v = jnp.var(x, axis=axis, keepdims=True)
    return (x - m) / jnp.sqrt(v + eps)
def _scatter_add(tgt, idx, src, axis=0):
    return tgt.at[idx].add(src)
def _segment_sum(src, seg, n):
    return jax.ops.segment_sum(src, seg, n)
class _Rng:
    def __init__(self, key):
        self._k = key
    def _next(self):
        self._k, sub = jax.random.split(self._k)
        return sub
    def normal(self, shape):
        return jax.random.normal(self._next(), shape, dtype=jnp.bfloat16)
    def randint(self, lo, hi, shape):
        return jax.random.randint(self._next(), shape, lo, hi, dtype=jnp.int32)
    def uniform(self, shape, lo=0.0, hi=1.0):
        return jax.random.uniform(self._next(), shape, jnp.bfloat16, lo, hi)
    def permutation(self, n):
        return jax.random.permutation(self._next(), n)


kernel_name = 'standalone__gqa_softmax__decode'

def setup_inputs():
    _rng = _Rng(jax.random.key(int.from_bytes(__import__("os").urandom(4), "little")))
    _w = (lambda a: (lambda t: t.astype(jnp.bfloat16) if jnp.issubdtype(t.dtype, jnp.floating) else t)(jnp.asarray(a)))
    B, Hq, Hkv, Sq, Sk, D = 8, 32, 32, 1, 4096, 128
    return {
        "q": _w((lambda *s: _rng.normal(s) * 0.4)(B, Hq, Sq, D)),
        "k": _w((lambda *s: _rng.normal(s) * 0.4)(B, Hkv, Sk, D)),
        "v": _w((lambda *s: _rng.normal(s) * 0.05)(B, Hkv, Sk, D)),
    }

def reference(q, k, v):
    B, Hq, Sq, D = q.shape
    Hkv = k.shape[1]
    rep = Hq // Hkv
    k = jnp.repeat(k, rep, axis=1)
    v = jnp.repeat(v, rep, axis=1)
    scale = D ** -0.5
    scores = jnp.einsum("bhqd,bhkd->bhqk", q, k) * scale
    p = _softmax(scores, axis=-1)
    return jnp.einsum("bhqk,bhkd->bhqd", p, v)
```

```python
import jax
import jax.numpy as jnp
from jax import lax
import jax.experimental.pallas as pl
import jax.experimental.pallas.tpu as pltpu

_NR = 4
_CH = 128
_W = 14
_NSEM = 16
_NSLOT = 4
_PRIOS = (1, 1, 1, 0)
_QK_EVERY = 2


@jax.jit
def pallas_standalone__gqa_softmax__decode_kernel(
    q: jax.Array,
    k: jax.Array,
    v: jax.Array,
):
    B, Hq, Sq, D = q.shape
    _, Hkv, Sk, _ = k.shape
    rep = Hq // Hkv
    M = rep * Sq
    G = B * Hkv
    NR, CH, W, NSEM, NSLOT = _NR, _CH, _W, _NSEM, _NSLOT
    prios, qk_every = _PRIOS, _QK_EVERY
    assert G % NR == 0 and Sk % (4 * CH) == 0
    scale = D ** -0.5
    NC = Sk // CH
    T = G // NR
    H1 = NC // 2
    H2 = (3 * NC) // 4
    assert W < NSEM and W <= NC and 1 + qk_every * NR <= H1

    q2 = q.reshape(G * M, D)
    k3 = k.reshape(G, Sk, D)
    v3 = v.reshape(G, Sk, D)

    def kernel(q_hbm, k_hbm, v_hbm, o_hbm, kbuf, vbuf, qbuf, q32, o32, obuf,
               pbuf, ksem, vsem, qsem, osem):
        def kcp(s, c, r, sem_i):
            row = pl.multiple_of(c * CH, CH)
            return pltpu.make_async_copy(
                k_hbm.at[s * NR + r, pl.ds(row, CH)],
                kbuf.at[s % NSLOT, r, pl.ds(row, CH)], ksem.at[sem_i])

        def vcp(s, c, r, sem_i):
            row = pl.multiple_of(c * CH, CH)
            return pltpu.make_async_copy(
                v_hbm.at[(s - 1) * NR + r, pl.ds(row, CH)],
                vbuf.at[(s - 1) % NSLOT, r, pl.ds(row, CH)], vsem.at[sem_i])

        def issue_static(s, c, sem_i, has_k, has_v):
            u = 0
            for r in range(NR):
                if has_k:
                    kcp(s, c, r, sem_i).start(priority=prios[u % len(prios)])
                    u += 1
                if has_v:
                    vcp(s, c, r, sem_i).start(priority=prios[u % len(prios)])
                    u += 1

        def issue(un):
            sn = un // NC
            cn = un % NC
            sem_i = un % NSEM

            @pl.when(jnp.logical_and(sn >= 1, sn < T))
            def _():
                issue_static(sn, cn, sem_i, True, True)

            @pl.when(sn == 0)
            def _():
                issue_static(sn, cn, sem_i, True, False)

            @pl.when(sn == T)
            def _():
                issue_static(sn, cn, sem_i, False, True)

        def wait(s, c):
            sem_i = (s * NC + c) % NSEM
            row = pl.multiple_of(c * CH, CH)

            @pl.when(s < T)
            def _():
                dst = kbuf.at[s % NSLOT, :, pl.ds(row, CH)]
                pltpu.make_async_copy(dst, dst, ksem.at[sem_i]).wait()

            @pl.when(s >= 1)
            def _():
                dst = vbuf.at[(s - 1) % NSLOT, :, pl.ds(row, CH)]
                pltpu.make_async_copy(dst, dst, vsem.at[sem_i]).wait()

        def units(s, c0, n):
            def body(i, _):
                c = c0 + i
                wait(s, c)
                issue(s * NC + c + W)
                return 0
            lax.fori_loop(0, n, body, 0)

        def qk_piece(grp, r):
            g = grp * NR + r
            qh = q32[pl.ds(g * M, M), :].astype(kbuf.dtype)
            s_ = lax.dot_general(
                qh, kbuf[grp % NSLOT, r], (((1,), (1,)), ((), ())),
                preferred_element_type=jnp.float32) * scale
            m = jnp.max(s_, axis=-1, keepdims=True)
            p = jnp.exp(s_ - m)
            l = jnp.sum(p, axis=-1, keepdims=True)
            pbuf[r] = p * (1.0 / l)

        def pv_part(grp, lo, hi, first):
            for r in range(NR):
                g = grp * NR + r
                p = pbuf[r, :, lo:hi].astype(vbuf.dtype)
                o = jnp.dot(p, vbuf[grp % NSLOT, r, lo:hi, :],
                            preferred_element_type=jnp.float32)
                if first:
                    o32[pl.ds(g * M, M), :] = o
                else:
                    o32[pl.ds(g * M, M), :] += o

        qcopy = pltpu.make_async_copy(q_hbm, qbuf, qsem)
        for un in range(W):
            issue_static(0, un, un % NSEM, True, False)
            if un == 0:
                qcopy.start()
        qcopy.wait()
        q32[...] = qbuf[...].astype(jnp.float32)

        def stage(s, _):
            units(s, 0, 1)

            @pl.when(s >= 2)
            def _():
                pv_part(s - 2, H2 * CH, NC * CH, False)

            def qkb(r, _):
                units(s, 1 + r * qk_every, qk_every)

                @pl.when(s >= 1)
                def _():
                    qk_piece(s - 1, r)
                return 0
            lax.fori_loop(0, NR, qkb, 0)
            c1 = 1 + qk_every * NR
            units(s, c1, H1 - c1)

            @pl.when(s >= 1)
            def _():
                pv_part(s - 1, 0, H1 * CH, True)
            units(s, H1, H2 - H1)

            @pl.when(s >= 1)
            def _():
                pv_part(s - 1, H1 * CH, H2 * CH, False)
            units(s, H2, NC - H2)
            return 0

        lax.fori_loop(0, T + 1, stage, 0)
        pv_part(T - 1, H2 * CH, NC * CH, False)
        obuf[...] = o32[...].astype(obuf.dtype)
        ocopy = pltpu.make_async_copy(obuf, o_hbm, osem)
        ocopy.start()
        ocopy.wait()

    out = pl.pallas_call(
        kernel,
        in_specs=[pl.BlockSpec(memory_space=pl.ANY)] * 3,
        out_specs=pl.BlockSpec(memory_space=pl.ANY),
        out_shape=jax.ShapeDtypeStruct((G * M, D), q.dtype),
        scratch_shapes=[
            pltpu.VMEM((NSLOT, NR, Sk, D), k.dtype),
            pltpu.VMEM((NSLOT, NR, Sk, D), v.dtype),
            pltpu.VMEM((G * M, D), q.dtype),
            pltpu.VMEM((G * M, D), jnp.float32),
            pltpu.VMEM((G * M, D), jnp.float32),
            pltpu.VMEM((G * M, D), q.dtype),
            pltpu.VMEM((NR, M, Sk), jnp.float32),
            pltpu.SemaphoreType.DMA((NSEM,)),
            pltpu.SemaphoreType.DMA((NSEM,)),
            pltpu.SemaphoreType.DMA(()),
            pltpu.SemaphoreType.DMA(()),
        ],
        compiler_params=pltpu.CompilerParams(
            vmem_limit_bytes=100 * 1024 * 1024,
            disable_bounds_checks=True,
        ),
    )(q2, k3, v3)
    return out.reshape(B, Hq, Sq, D)
```

```python
import jax
import jax.numpy as jnp
from jax import lax
import jax.experimental.pallas as pl
import jax.experimental.pallas.tpu as pltpu

_NR = 8
_CH = 128
_OFF = 104
_W = 12
_NSEM = 16
_NSLOT = 4
_PRIOS = (1, 1, 1, 0)
_QK_EVERY = 2


@jax.jit
def pallas_standalone__gqa_softmax__decode_kernel(
    q: jax.Array,
    k: jax.Array,
    v: jax.Array,
):
    B, Hq, Sq, D = q.shape
    _, Hkv, Sk, _ = k.shape
    rep = Hq // Hkv
    M = rep * Sq
    G = B * Hkv
    NR, CH, OFF, W, NSEM, NSLOT = _NR, _CH, _OFF, _W, _NSEM, _NSLOT
    prios, qk_every = _PRIOS, _QK_EVERY
    assert G % NR == 0 and Sk % (4 * CH) == 0
    scale = D ** -0.5
    NC = Sk // CH
    T = G // NR
    H1 = NC // 2
    H2 = (3 * NC) // 4
    C1 = 1 + qk_every * NR
    CF = NC - W
    assert W < NSEM and C1 <= H1 + 1 and C1 <= CF < NC
    pieces0 = ([(0, OFF)] if OFF else []) + [(Sk - (CH - OFF), CH - OFF)]

    q2 = q.reshape(G * M, D)
    k3 = k.reshape(G, Sk, D)
    v3 = v.reshape(G, Sk, D)

    def kernel(q_hbm, k_hbm, v_hbm, o_hbm, kbuf, vbuf, qbuf, q32, o32, obuf,
               pbuf, ksem, vsem, qsem, osem):
        def kcp(s, row, n, r, sem_i):
            return pltpu.make_async_copy(
                k_hbm.at[s * NR + r, pl.ds(row, n)],
                kbuf.at[s % NSLOT, r, pl.ds(row, n)], ksem.at[sem_i])

        def vcp(s, row, n, r, sem_i):
            return pltpu.make_async_copy(
                v_hbm.at[(s - 1) * NR + r, pl.ds(row, n)],
                vbuf.at[(s - 1) % NSLOT, r, pl.ds(row, n)], vsem.at[sem_i])

        def unit_pieces(c, first):
            if first:
                return pieces0
            return [(pl.multiple_of(OFF + (c - 1) * CH, 8), CH)]

        def issue_static(s, c, sem_i, has_k, has_v, first):
            u = 0
            for (row, n) in unit_pieces(c, first):
                for r in range(NR):
                    if has_k:
                        kcp(s, row, n, r, sem_i).start(
                            priority=prios[u % len(prios)])
                        u += 1
                    if has_v:
                        vcp(s, row, n, r, sem_i).start(
                            priority=prios[u % len(prios)])
                        u += 1

        def issue(un, first):
            sn = un // NC
            cn = un % NC
            sem_i = un % NSEM

            @pl.when(jnp.logical_and(sn >= 1, sn < T))
            def _():
                issue_static(sn, cn, sem_i, True, True, first)

            @pl.when(sn == 0)
            def _():
                issue_static(sn, cn, sem_i, True, False, first)

            @pl.when(sn == T)
            def _():
                issue_static(sn, cn, sem_i, False, True, first)

        def wait(s, c, first):
            sem_i = (s * NC + c) % NSEM

            @pl.when(s < T)
            def _():
                for (row, n) in unit_pieces(c, first):
                    dst = kbuf.at[s % NSLOT, :, pl.ds(row, n)]
                    pltpu.make_async_copy(dst, dst, ksem.at[sem_i]).wait()

            @pl.when(s >= 1)
            def _():
                for (row, n) in unit_pieces(c, first):
                    dst = vbuf.at[(s - 1) % NSLOT, :, pl.ds(row, n)]
                    pltpu.make_async_copy(dst, dst, vsem.at[sem_i]).wait()

        def unit(s, c, wfirst, ifirst):
            wait(s, c, wfirst)
            issue(s * NC + c + W, ifirst)

        def units(s, c0, c1):
            segs = []
            a = c0
            for sp in sorted({0, CF}):
                if a <= sp < c1:
                    if sp > a:
                        segs.append((a, sp))
                    segs.append((sp, sp + 1))
                    a = sp + 1
            if a < c1:
                segs.append((a, c1))
            for (x, y) in segs:
                if y - x == 1:
                    unit(s, x, x == 0, x == CF)
                else:
                    def body(c, _):
                        unit(s, c, False, False)
                        return 0
                    lax.fori_loop(x, y, body, 0)

        def qk_piece(grp, r):
            g = grp * NR + r
            qh = q32[pl.ds(g * M, M), :].astype(kbuf.dtype)
            s_ = lax.dot_general(
                qh, kbuf[grp % NSLOT, r], (((1,), (1,)), ((), ())),
                preferred_element_type=jnp.float32) * scale
            m = jnp.max(s_, axis=-1, keepdims=True)
            p = jnp.exp(s_ - m)
            l = jnp.sum(p, axis=-1, keepdims=True)
            pbuf[r] = p * (1.0 / l)

        def pv_part(grp, lo, hi, first):
            for r in range(NR):
                g = grp * NR + r
                p = pbuf[r, :, lo:hi].astype(vbuf.dtype)
                o = jnp.dot(p, vbuf[grp % NSLOT, r, lo:hi, :],
                            preferred_element_type=jnp.float32)
                if first:
                    o32[pl.ds(g * M, M), :] = o
                else:
                    o32[pl.ds(g * M, M), :] += o

        qcopy = pltpu.make_async_copy(q_hbm, qbuf, qsem)
        for un in range(W):
            issue_static(0, un, un % NSEM, True, False, un == 0)
            if un == 0:
                qcopy.start()
        qcopy.wait()
        q32[...] = qbuf[...].astype(jnp.float32)

        def stage(s, _):
            units(s, 0, 1)

            @pl.when(s >= 2)
            def _():
                pv_part(s - 2, H2 * CH, NC * CH, False)

            def qkb(r, _):
                def body(i, _):
                    unit(s, 1 + r * qk_every + i, False, False)
                    return 0
                lax.fori_loop(0, qk_every, body, 0)

                @pl.when(s >= 1)
                def _():
                    qk_piece(s - 1, r)
                return 0
            lax.fori_loop(0, NR, qkb, 0)
            units(s, C1, H1 + 1)

            @pl.when(s >= 1)
            def _():
                pv_part(s - 1, 0, H1 * CH, True)
            units(s, H1 + 1, H2 + 1)

            @pl.when(s >= 1)
            def _():
                pv_part(s - 1, H1 * CH, H2 * CH, False)
            units(s, H2 + 1, NC)
            return 0

        lax.fori_loop(0, T + 1, stage, 0)
        pv_part(T - 1, H2 * CH, NC * CH, False)
        obuf[...] = o32[...].astype(obuf.dtype)
        ocopy = pltpu.make_async_copy(obuf, o_hbm, osem)
        ocopy.start()
        ocopy.wait()

    out = pl.pallas_call(
        kernel,
        in_specs=[pl.BlockSpec(memory_space=pl.ANY)] * 3,
        out_specs=pl.BlockSpec(memory_space=pl.ANY),
        out_shape=jax.ShapeDtypeStruct((G * M, D), q.dtype),
        scratch_shapes=[
            pltpu.VMEM((NSLOT, NR, Sk, D), k.dtype),
            pltpu.VMEM((NSLOT, NR, Sk, D), v.dtype),
            pltpu.VMEM((G * M, D), q.dtype),
            pltpu.VMEM((G * M, D), jnp.float32),
            pltpu.VMEM((G * M, D), jnp.float32),
            pltpu.VMEM((G * M, D), q.dtype),
            pltpu.VMEM((NR, M, Sk), jnp.float32),
            pltpu.SemaphoreType.DMA((NSEM,)),
            pltpu.SemaphoreType.DMA((NSEM,)),
            pltpu.SemaphoreType.DMA(()),
            pltpu.SemaphoreType.DMA(()),
        ],
        compiler_params=pltpu.CompilerParams(
            vmem_limit_bytes=100 * 1024 * 1024,
            disable_bounds_checks=True,
        ),
    )(q2, k3, v3)
    return out.reshape(B, Hq, Sq, D)
```

```python
import jax
import jax.numpy as jnp
from jax import lax
import jax.experimental.pallas as pl
import jax.experimental.pallas.tpu as pltpu

_NR = 8
_HS = 4
_CH = 128
_OFF = 104
_W = 12
_NSEM = 16
_NSLOT = 4
_PRIOS = (1, 1, 1, 0)
_QK_EVERY = 2
_PARTS = (16, 24, 28)


@jax.jit
def pallas_standalone__gqa_softmax__decode_kernel(
    q: jax.Array,
    k: jax.Array,
    v: jax.Array,
):
    B, Hq, Sq, D = q.shape
    _, Hkv, Sk, _ = k.shape
    rep = Hq // Hkv
    M = rep * Sq
    G = B * Hkv
    NR, HS, CH, OFF, W, NSEM, NSLOT = _NR, _HS, _CH, _OFF, _W, _NSEM, _NSLOT
    prios, qk_every = _PRIOS, _QK_EVERY
    assert k.dtype == v.dtype and G % (NR * HS) == 0 and Sk % CH == 0
    scale = D ** -0.5
    NC = Sk // CH
    T = G // NR
    C1 = 1 + qk_every * NR
    CF = NC - W
    bounds = (0,) + tuple(_PARTS) + (NC,)
    NP = len(bounds) - 1
    assert W < NSEM and C1 <= bounds[1] + 1 and C1 <= CF < NC
    assert bounds[-2] < NC
    pieces0 = ([(0, OFF)] if OFF else []) + [(Sk - (CH - OFF), CH - OFF)]

    def head_of(t, r):
        return (t // HS) * (NR * HS) + r * HS + (t % HS)

    q2 = q.reshape(G * M, D)
    k3 = k.reshape(G, Sk, D)
    v3 = v.reshape(G, Sk, D)

    def kernel(q_hbm, k_hbm, v_hbm, o_hbm, kvbuf, qbuf, q32, o32, obuf, pbuf,
               sem, qsem, osem):
        kbuf = kvbuf.at[0]
        vbuf = kvbuf.at[1]

        def unit_pieces(c, first):
            if first:
                return pieces0
            return [(pl.multiple_of(OFF + (c - 1) * CH, 8), CH)]

        def issue_arr(hbm, buf, t, c, sem_i, first):
            h0 = head_of(t, 0)
            slot = t % NSLOT
            for (row, n) in unit_pieces(c, first):
                for r in range(NR):
                    pltpu.make_async_copy(
                        hbm.at[h0 + r * HS, pl.ds(row, n)],
                        buf.at[slot, r, pl.ds(row, n)],
                        sem.at[sem_i],
                    ).start(priority=prios[r % len(prios)])

        def issue(un, first):
            sn = un // NC
            cn = un % NC
            sem_i = un % NSEM

            @pl.when(sn < T)
            def _():
                issue_arr(k_hbm, kbuf, sn, cn, sem_i, first)

            @pl.when(jnp.logical_and(sn >= 1, sn <= T))
            def _():
                issue_arr(v_hbm, vbuf, sn - 1, cn, sem_i, first)

        def wait(s, c, first):
            sem_i = (s * NC + c) % NSEM

            @pl.when(s < T)
            def _():
                for (row, n) in unit_pieces(c, first):
                    dst = kbuf.at[s % NSLOT, :, pl.ds(row, n)]
                    pltpu.make_async_copy(dst, dst, sem.at[sem_i]).wait()

            @pl.when(s >= 1)
            def _():
                for (row, n) in unit_pieces(c, first):
                    dst = vbuf.at[(s - 1) % NSLOT, :, pl.ds(row, n)]
                    pltpu.make_async_copy(dst, dst, sem.at[sem_i]).wait()

        def unit(s, c, wfirst, ifirst):
            wait(s, c, wfirst)
            issue(s * NC + c + W, ifirst)

        def units(s, c0, c1):
            segs = []
            a = c0
            for sp in sorted({0, CF}):
                if a <= sp < c1:
                    if sp > a:
                        segs.append((a, sp))
                    segs.append((sp, sp + 1))
                    a = sp + 1
            if a < c1:
                segs.append((a, c1))
            for (x, y) in segs:
                if y - x == 1:
                    unit(s, x, x == 0, x == CF)
                else:
                    def body(c, _):
                        unit(s, c, False, False)
                        return 0
                    lax.fori_loop(x, y, body, 0)

        def qk_piece(grp, r):
            g = head_of(grp, r)
            qh = q32[pl.ds(g * M, M), :].astype(kvbuf.dtype)
            s_ = lax.dot_general(
                qh, kbuf[grp % NSLOT, r], (((1,), (1,)), ((), ())),
                preferred_element_type=jnp.float32) * scale
            m = jnp.max(s_, axis=-1, keepdims=True)
            p = jnp.exp(s_ - m)
            l = jnp.sum(p, axis=-1, keepdims=True)
            pbuf[r] = p * (1.0 / l)

        def pv_part(grp, i):
            lo, hi = bounds[i] * CH, bounds[i + 1] * CH
            for r in range(NR):
                g = head_of(grp, r)
                p = pbuf[r, :, lo:hi].astype(kvbuf.dtype)
                o = jnp.dot(p, vbuf[grp % NSLOT, r, lo:hi, :],
                            preferred_element_type=jnp.float32)
                if i == 0:
                    o32[pl.ds(g * M, M), :] = o
                else:
                    o32[pl.ds(g * M, M), :] += o

        qcopy = pltpu.make_async_copy(q_hbm, qbuf, qsem)
        for un in range(W):
            issue_arr(k_hbm, kbuf, 0, un, un % NSEM, un == 0)
            if un == 0:
                qcopy.start()
        qcopy.wait()
        q32[...] = qbuf[...].astype(jnp.float32)

        def stage(s, _):
            units(s, 0, 1)

            @pl.when(s >= 2)
            def _():
                pv_part(s - 2, NP - 1)

            def qkb(r, _):
                def body(i, _):
                    unit(s, 1 + r * qk_every + i, False, False)
                    return 0
                lax.fori_loop(0, qk_every, body, 0)

                @pl.when(s >= 1)
                def _():
                    qk_piece(s - 1, r)
                return 0
            lax.fori_loop(0, NR, qkb, 0)
            a = C1
            for i in range(NP - 1):
                units(s, a, bounds[i + 1] + 1)
                a = bounds[i + 1] + 1

                @pl.when(s >= 1)
                def _(i=i):
                    pv_part(s - 1, i)
            units(s, a, NC)
            return 0

        lax.fori_loop(0, T + 1, stage, 0)
        pv_part(T - 1, NP - 1)
        obuf[...] = o32[...].astype(obuf.dtype)
        ocopy = pltpu.make_async_copy(obuf, o_hbm, osem)
        ocopy.start()
        ocopy.wait()

    out = pl.pallas_call(
        kernel,
        in_specs=[pl.BlockSpec(memory_space=pl.ANY)] * 3,
        out_specs=pl.BlockSpec(memory_space=pl.ANY),
        out_shape=jax.ShapeDtypeStruct((G * M, D), q.dtype),
        scratch_shapes=[
            pltpu.VMEM((2, NSLOT, NR, Sk, D), k.dtype),
            pltpu.VMEM((G * M, D), q.dtype),
            pltpu.VMEM((G * M, D), jnp.float32),
            pltpu.VMEM((G * M, D), jnp.float32),
            pltpu.VMEM((G * M, D), q.dtype),
            pltpu.VMEM((NR, M, Sk), jnp.float32),
            pltpu.SemaphoreType.DMA((NSEM,)),
            pltpu.SemaphoreType.DMA(()),
            pltpu.SemaphoreType.DMA(()),
        ],
        compiler_params=pltpu.CompilerParams(
            vmem_limit_bytes=100 * 1024 * 1024,
            disable_bounds_checks=True,
        ),
    )(q2, k3, v3)
    return out.reshape(B, Hq, Sq, D)
```

```python
import jax
import jax.numpy as jnp
from jax import lax
import jax.experimental.pallas as pl
import jax.experimental.pallas.tpu as pltpu

_NR = 8
_HS = 4
_CH = 128
_OFF = 104
_W = 12
_NSEM = 16
_NSLOT = 4
_PRIOS = (1, 1, 1, 0)
_QK_EVERY = 2
_PARTS = (16, 24, 28)


@jax.jit
def pallas_standalone__gqa_softmax__decode_kernel(
    q: jax.Array,
    k: jax.Array,
    v: jax.Array,
):
    B, Hq, Sq, D = q.shape
    _, Hkv, Sk, _ = k.shape
    rep = Hq // Hkv
    M = rep * Sq
    G = B * Hkv
    NR, HS, CH, OFF, W, NSEM, NSLOT = _NR, _HS, _CH, _OFF, _W, _NSEM, _NSLOT
    prios, qk_every = _PRIOS, _QK_EVERY
    assert k.dtype == v.dtype and G % (NR * HS) == 0 and Sk % CH == 0
    scale = D ** -0.5
    NC = Sk // CH
    T = G // NR
    C1 = 1 + qk_every * NR
    CF = NC - W
    bounds = (0,) + tuple(_PARTS) + (NC,)
    NP = len(bounds) - 1
    assert W < NSEM and C1 <= bounds[1] + 1 and C1 <= CF < NC
    assert bounds[-2] < NC
    pieces0 = ([(0, OFF)] if OFF else []) + [(Sk - (CH - OFF), CH - OFF)]

    def head_of(t, r):
        return (t // HS) * (NR * HS) + r * HS + (t % HS)

    q2 = q.reshape(G * M, D)
    k3 = k.reshape(G, Sk, D)
    v3 = v.reshape(G, Sk, D)

    def kernel(q_hbm, k_hbm, v_hbm, o_hbm, kvbuf, qbuf, q32, o32, obuf, pbuf,
               sem, qsem, osem):
        kbuf = kvbuf.at[0]
        vbuf = kvbuf.at[1]

        def unit_pieces(c, first):
            if first:
                return pieces0
            return [(pl.multiple_of(OFF + (c - 1) * CH, 8), CH)]

        def issue_arr(hbm, buf, t, c, sem_i, first):
            h0 = head_of(t, 0)
            slot = t % NSLOT
            for (row, n) in unit_pieces(c, first):
                for r in range(NR):
                    pltpu.make_async_copy(
                        hbm.at[h0 + r * HS, pl.ds(row, n)],
                        buf.at[slot, r, pl.ds(row, n)],
                        sem.at[sem_i],
                    ).start(priority=prios[r % len(prios)])

        def issue(un, first):
            sn = un // NC
            cn = un % NC
            sem_i = un % NSEM

            @pl.when(sn < T)
            def _():
                issue_arr(k_hbm, kbuf, sn, cn, sem_i, first)

            @pl.when(jnp.logical_and(sn >= 1, sn <= T))
            def _():
                issue_arr(v_hbm, vbuf, sn - 1, cn, NSEM + sem_i, first)

        def wait(s, c, first):
            sem_i = (s * NC + c) % NSEM

            @pl.when(s < T)
            def _():
                for (row, n) in unit_pieces(c, first):
                    dst = kbuf.at[s % NSLOT, :, pl.ds(row, n)]
                    pltpu.make_async_copy(dst, dst, sem.at[sem_i]).wait()

            @pl.when(s >= 1)
            def _():
                for (row, n) in unit_pieces(c, first):
                    dst = vbuf.at[(s - 1) % NSLOT, :, pl.ds(row, n)]
                    pltpu.make_async_copy(
                        dst, dst, sem.at[NSEM + sem_i]).wait()

        def unit(s, c, wfirst, ifirst):
            wait(s, c, wfirst)
            issue(s * NC + c + W, ifirst)

        def units(s, c0, c1):
            segs = []
            a = c0
            for sp in sorted({0, CF}):
                if a <= sp < c1:
                    if sp > a:
                        segs.append((a, sp))
                    segs.append((sp, sp + 1))
                    a = sp + 1
            if a < c1:
                segs.append((a, c1))
            for (x, y) in segs:
                if y - x == 1:
                    unit(s, x, x == 0, x == CF)
                else:
                    def body(c, _):
                        unit(s, c, False, False)
                        return 0
                    lax.fori_loop(x, y, body, 0)

        def qk_piece(grp, r):
            g = head_of(grp, r)
            qh = q32[pl.ds(g * M, M), :].astype(kvbuf.dtype)
            s_ = lax.dot_general(
                qh, kbuf[grp % NSLOT, r], (((1,), (1,)), ((), ())),
                preferred_element_type=jnp.float32) * scale
            m = jnp.max(s_, axis=-1, keepdims=True)
            p = jnp.exp(s_ - m)
            l = jnp.sum(p, axis=-1, keepdims=True)
            pbuf[r] = p * (1.0 / l)

        def pv_part(grp, i):
            lo, hi = bounds[i] * CH, bounds[i + 1] * CH
            for r in range(NR):
                g = head_of(grp, r)
                p = pbuf[r, :, lo:hi].astype(kvbuf.dtype)
                o = jnp.dot(p, vbuf[grp % NSLOT, r, lo:hi, :],
                            preferred_element_type=jnp.float32)
                if i == 0:
                    o32[pl.ds(g * M, M), :] = o
                else:
                    o32[pl.ds(g * M, M), :] += o

        qcopy = pltpu.make_async_copy(q_hbm, qbuf, qsem)
        for un in range(W):
            issue_arr(k_hbm, kbuf, 0, un, un % NSEM, un == 0)
            if un == 0:
                qcopy.start()

        def stage(s, _):
            units(s, 0, 1)

            @pl.when(s == 1)
            def _():
                qcopy.wait()
                q32[...] = qbuf[...].astype(jnp.float32)

            @pl.when(s >= 2)
            def _():
                pv_part(s - 2, NP - 1)

            def qkb(r, _):
                def body(i, _):
                    unit(s, 1 + r * qk_every + i, False, False)
                    return 0
                lax.fori_loop(0, qk_every, body, 0)

                @pl.when(s >= 1)
                def _():
                    qk_piece(s - 1, r)
                return 0
            lax.fori_loop(0, NR, qkb, 0)
            a = C1
            for i in range(NP - 1):
                units(s, a, bounds[i + 1] + 1)
                a = bounds[i + 1] + 1

                @pl.when(s >= 1)
                def _(i=i):
                    pv_part(s - 1, i)
            units(s, a, NC)
            return 0

        lax.fori_loop(0, T + 1, stage, 0)
        pv_part(T - 1, NP - 1)
        obuf[...] = o32[...].astype(obuf.dtype)
        ocopy = pltpu.make_async_copy(obuf, o_hbm, osem)
        ocopy.start()
        ocopy.wait()

    out = pl.pallas_call(
        kernel,
        in_specs=[pl.BlockSpec(memory_space=pl.ANY)] * 3,
        out_specs=pl.BlockSpec(memory_space=pl.ANY),
        out_shape=jax.ShapeDtypeStruct((G * M, D), q.dtype),
        scratch_shapes=[
            pltpu.VMEM((2, NSLOT, NR, Sk, D), k.dtype),
            pltpu.VMEM((G * M, D), q.dtype),
            pltpu.VMEM((G * M, D), jnp.float32),
            pltpu.VMEM((G * M, D), jnp.float32),
            pltpu.VMEM((G * M, D), q.dtype),
            pltpu.VMEM((NR, M, Sk), jnp.float32),
            pltpu.SemaphoreType.DMA((2 * NSEM,)),
            pltpu.SemaphoreType.DMA(()),
            pltpu.SemaphoreType.DMA(()),
        ],
        compiler_params=pltpu.CompilerParams(
            vmem_limit_bytes=100 * 1024 * 1024,
            disable_bounds_checks=True,
        ),
    )(q2, k3, v3)
    return out.reshape(B, Hq, Sq, D)
```

```python
import jax
import jax.numpy as jnp
from jax import lax
import jax.experimental.pallas as pl
import jax.experimental.pallas.tpu as pltpu

_NR = 8
_HS = 4
_CH = 128
_OFF = 104
_W = 12
_NSEM = 16
_NSLOT = 4
_PRIOS = (0, 1, 1, 1)
_QK_EVERY = 2
_PARTS = (16, 24, 28)


@jax.jit
def pallas_standalone__gqa_softmax__decode_kernel(
    q: jax.Array,
    k: jax.Array,
    v: jax.Array,
):
    B, Hq, Sq, D = q.shape
    _, Hkv, Sk, _ = k.shape
    rep = Hq // Hkv
    M = rep * Sq
    G = B * Hkv
    NR, HS, CH, OFF, W, NSEM, NSLOT = _NR, _HS, _CH, _OFF, _W, _NSEM, _NSLOT
    prios, qk_every = _PRIOS, _QK_EVERY
    assert k.dtype == v.dtype and G % (NR * HS) == 0 and Sk % CH == 0
    scale = D ** -0.5
    NC = Sk // CH
    T = G // NR
    C1 = 1 + qk_every * NR
    CF = NC - W
    bounds = (0,) + tuple(_PARTS) + (NC,)
    NP = len(bounds) - 1
    assert W < NSEM and C1 <= bounds[1] + 1 and C1 <= CF < NC
    assert bounds[-2] < NC
    pieces0 = ([(0, OFF)] if OFF else []) + [(Sk - (CH - OFF), CH - OFF)]

    def head_of(t, r):
        return (t // HS) * (NR * HS) + r * HS + (t % HS)

    q2 = q.reshape(G * M, D)
    k3 = k.reshape(G, Sk, D)
    v3 = v.reshape(G, Sk, D)

    def kernel(q_hbm, k_hbm, v_hbm, o_hbm, kvbuf, qbuf, q32, o32, obuf, pbuf,
               sem, qsem, osem):
        kbuf = kvbuf.at[0]
        vbuf = kvbuf.at[1]

        def unit_pieces(c, first):
            if first:
                return pieces0
            return [(pl.multiple_of(OFF + (c - 1) * CH, 8), CH)]

        def copies(hbm, buf, t, c, sem_i, first):
            h0 = head_of(t, 0)
            slot = t % NSLOT
            return [
                (pltpu.make_async_copy(
                    hbm.at[h0 + r * HS, pl.ds(row, n)],
                    buf.at[slot, r, pl.ds(row, n)],
                    sem.at[sem_i]), prios[r % len(prios)])
                for (row, n) in unit_pieces(c, first) for r in range(NR)]

        def issue_arr(hbm, buf, t, c, sem_i, first):
            for cp, prio in copies(hbm, buf, t, c, sem_i, first):
                cp.start(priority=prio)

        def wait_arr(hbm, buf, t, c, sem_i, first):
            if first:
                for cp, _ in copies(hbm, buf, t, c, sem_i, first):
                    cp.wait()
            else:
                ((row, n),) = unit_pieces(c, first)
                dst = buf.at[t % NSLOT, :, pl.ds(row, n)]
                pltpu.make_async_copy(dst, dst, sem.at[sem_i]).wait()

        def issue(un, first):
            sn = un // NC
            cn = un % NC
            sem_i = un % NSEM

            @pl.when(sn < T)
            def _():
                issue_arr(k_hbm, kbuf, sn, cn, sem_i, first)

            @pl.when(jnp.logical_and(sn >= 1, sn <= T))
            def _():
                issue_arr(v_hbm, vbuf, sn - 1, cn, NSEM + sem_i, first)

        def wait(s, c, first):
            sem_i = (s * NC + c) % NSEM

            @pl.when(s < T)
            def _():
                wait_arr(k_hbm, kbuf, s, c, sem_i, first)

            @pl.when(s >= 1)
            def _():
                wait_arr(v_hbm, vbuf, s - 1, c, NSEM + sem_i, first)

        def unit(s, c, wfirst, ifirst):
            wait(s, c, wfirst)
            issue(s * NC + c + W, ifirst)

        def units(s, c0, c1):
            segs = []
            a = c0
            for sp in sorted({0, CF}):
                if a <= sp < c1:
                    if sp > a:
                        segs.append((a, sp))
                    segs.append((sp, sp + 1))
                    a = sp + 1
            if a < c1:
                segs.append((a, c1))
            for (x, y) in segs:
                if y - x == 1:
                    unit(s, x, x == 0, x == CF)
                else:
                    def body(c, _):
                        unit(s, c, False, False)
                        return 0
                    lax.fori_loop(x, y, body, 0)

        def qk_piece(grp, r):
            g = head_of(grp, r)
            qh = q32[pl.ds(g * M, M), :].astype(kvbuf.dtype)
            s_ = lax.dot_general(
                qh, kbuf[grp % NSLOT, r], (((1,), (1,)), ((), ())),
                preferred_element_type=jnp.float32) * scale
            m = jnp.max(s_, axis=-1, keepdims=True)
            p = jnp.exp(s_ - m)
            l = jnp.sum(p, axis=-1, keepdims=True)
            pbuf[r] = p * (1.0 / l)

        def pv_part(grp, i):
            lo, hi = bounds[i] * CH, bounds[i + 1] * CH
            for r in range(NR):
                g = head_of(grp, r)
                p = pbuf[r, :, lo:hi].astype(kvbuf.dtype)
                o = jnp.dot(p, vbuf[grp % NSLOT, r, lo:hi, :],
                            preferred_element_type=jnp.float32)
                if i == 0:
                    o32[pl.ds(g * M, M), :] = o
                else:
                    o32[pl.ds(g * M, M), :] += o

        qcopy = pltpu.make_async_copy(q_hbm, qbuf, qsem)
        for un in range(W):
            issue_arr(k_hbm, kbuf, 0, un, un % NSEM, un == 0)
            if un == 0:
                qcopy.start()

        def stage(s, _):
            units(s, 0, 1)

            @pl.when(s == 1)
            def _():
                qcopy.wait()
                q32[...] = qbuf[...].astype(jnp.float32)

            @pl.when(s >= 2)
            def _():
                pv_part(s - 2, NP - 1)

            def qkb(r, _):
                def body(i, _):
                    unit(s, 1 + r * qk_every + i, False, False)
                    return 0
                lax.fori_loop(0, qk_every, body, 0)

                @pl.when(s >= 1)
                def _():
                    qk_piece(s - 1, r)
                return 0
            lax.fori_loop(0, NR, qkb, 0)
            a = C1
            for i in range(NP - 1):
                units(s, a, bounds[i + 1] + 1)
                a = bounds[i + 1] + 1

                @pl.when(s >= 1)
                def _(i=i):
                    pv_part(s - 1, i)
            units(s, a, NC)
            return 0

        lax.fori_loop(0, T + 1, stage, 0)
        pv_part(T - 1, NP - 1)
        obuf[...] = o32[...].astype(obuf.dtype)
        ocopy = pltpu.make_async_copy(obuf, o_hbm, osem)
        ocopy.start()
        ocopy.wait()

    out = pl.pallas_call(
        kernel,
        in_specs=[pl.BlockSpec(memory_space=pl.ANY)] * 3,
        out_specs=pl.BlockSpec(memory_space=pl.ANY),
        out_shape=jax.ShapeDtypeStruct((G * M, D), q.dtype),
        scratch_shapes=[
            pltpu.VMEM((2, NSLOT, NR, Sk, D), k.dtype),
            pltpu.VMEM((G * M, D), q.dtype),
            pltpu.VMEM((G * M, D), jnp.float32),
            pltpu.VMEM((G * M, D), jnp.float32),
            pltpu.VMEM((G * M, D), q.dtype),
            pltpu.VMEM((NR, M, Sk), jnp.float32),
            pltpu.SemaphoreType.DMA((2 * NSEM,)),
            pltpu.SemaphoreType.DMA(()),
            pltpu.SemaphoreType.DMA(()),
        ],
        compiler_params=pltpu.CompilerParams(
            vmem_limit_bytes=100 * 1024 * 1024,
            disable_bounds_checks=True,
        ),
    )(q2, k3, v3)
    return out.reshape(B, Hq, Sq, D)
```
